```python
import os as _os
_os.environ.setdefault('JAX_PLATFORMS', 'cpu')
import jax
import jax.numpy as jnp

def _softmax(x, axis=-1):
    return jax.nn.softmax(x, axis=axis)

def _gelu(x):
    return jax.nn.gelu(x, approximate=True)

def _silu(x):
    return jax.nn.silu(x)

def _sigmoid(x):
    return jax.nn.sigmoid(x)

def _layernorm(x, axis=-1, eps=1e-05):
    m = jnp.mean(x, axis=axis, keepdims=True)
    v = jnp.var(x, axis=axis, keepdims=True)
    return (x - m) / jnp.sqrt(v + eps)

def _scatter_add(tgt, idx, src, axis=0):
    return tgt.at[idx].add(src)

def _segment_sum(src, seg, n):
    return jax.ops.segment_sum(src, seg, n)

class _Rng:

    def __init__(self, key):
        self._k = key

    def _next(self):
        self._k, sub = jax.random.split(self._k)
        return sub

    def normal(self, shape):
        return jax.random.normal(self._next(), shape, dtype=jnp.bfloat16)

    def randint(self, lo, hi, shape):
        return jax.random.randint(self._next(), shape, lo, hi, dtype=jnp.int32)

    def uniform(self, shape, lo=0.0, hi=1.0):
        return jax.random.uniform(self._next(), shape, jnp.bfloat16, lo, hi)

    def permutation(self, n):
        return jax.random.permutation(self._next(), n)
kernel_name = 'adaLN_cond__sliding_local_dilated__mixer_channel_mlp__prompt'

def setup_inputs():
    _rng = _Rng(jax.random.key(int.from_bytes(__import__("os").urandom(4), "little")))
    _w = lambda a: (lambda t: t.astype(jnp.bfloat16) if jnp.issubdtype(t.dtype, jnp.floating) else t)(jnp.asarray(a))

    def _A_setup():
        B, S, D = (1, 2048, 512)
        return {'x': _w((lambda *s: _rng.normal(s) * 0.05)(B, S, D)), 'wqkv': _w((lambda *s: _rng.normal(s) * 0.05)(D, 3 * D)), 'wo': _w((lambda *s: _rng.normal(s) * 0.05)(D, D))}
    _A_in = _A_setup()

    def _B_setup():
        B, S, D, F = (1, 2048, 512, 1792)
        return {'x': _w((lambda *s: _rng.normal(s) * 0.05)(B, S, D)), 'w1': _w((lambda *s: _rng.normal(s) * 0.8)(D, F) * D ** (-0.5)), 'b1': _w((lambda *s: _rng.normal(s) * 0.8)(F)), 'w2': _w((lambda *s: _rng.normal(s) * 0.8)(F, D) * F ** (-0.5)), 'b2': _w((lambda *s: _rng.normal(s) * 0.4)(D))}
    _B_in = _B_setup()
    return {'A_x': _A_in['x'], 'A_wqkv': _A_in['wqkv'], 'A_wo': _A_in['wo'], 'B_x': _B_in['x'], 'B_w1': _B_in['w1'], 'B_b1': _B_in['b1'], 'B_w2': _B_in['w2'], 'B_b2': _B_in['b2'], 'c': _w((lambda *s: _rng.normal(s) * 0.05)(1, 512) * 8.0), 'w_mod': _w((lambda *s: _rng.normal(s) * 0.05)(512, 6 * 512) * 512 ** (-0.5) * 8.0)}

def reference(A_x, A_wqkv, A_wo, B_x, B_w1, B_b1, B_w2, B_b2, c, w_mod):

    def _A_ref(x, wqkv, wo):
        B, S, D = x.shape
        H = 32
        Dh = D // H
        W, dil = (8, 2)
        qkv = (lambda x, *d: x.transpose(*d))((x @ wqkv).reshape(B, S, 3, H, Dh), 2, 0, 3, 1, 4)
        q, k, v = (qkv[0], qkv[1], qkv[2])
        scale = Dh ** (-0.5)
        pos = jnp.arange(S)
        off = jnp.arange(W) * dil
        idx = pos[:, None] - off[None, :]
        mask = idx >= 0
        idx_c = jnp.where(mask, idx, 0).reshape(-1)
        kg = k[:, :, idx_c, :].reshape(B, H, S, W, Dh)
        vg = v[:, :, idx_c, :].reshape(B, H, S, W, Dh)
        logits = jnp.einsum('bhsd,bhswd->bhsw', q, kg) * scale
        logits = jnp.where(mask[None, None, :, :], logits, -1000000000.0)
        attn = _softmax(logits, axis=-1)
        o = jnp.einsum('bhsw,bhswd->bhsd', attn, vg)
        return (lambda x, *d: x.transpose(*d))(o, 0, 2, 1, 3).reshape(B, S, D) @ wo

    def _B_ref(x, w1, b1, w2, b2):
        y = _layernorm(x, axis=-1)
        h = _gelu(jnp.einsum('bsd,df->bsf', y, w1) + b1)
        return jnp.einsum('bsf,fd->bsd', h, w2) + b2
    x = A_x
    mod = (_silu(c) @ w_mod).reshape(c.shape[0], 6, 1, -1)
    sa, ca, ga, sb, cb, gb = (mod[:, 0].copy(), mod[:, 1].copy(), mod[:, 2].copy(), mod[:, 3].copy(), mod[:, 4].copy(), mod[:, 5].copy())
    h = _layernorm(x, axis=-1) * (1 + ca) + sa
    x = x + ga * _A_ref(h, A_wqkv, A_wo)
    h = _layernorm(x, axis=-1) * (1 + cb) + sb
    x = x + gb * _B_ref(h, B_w1, B_b1, B_w2, B_b2)
    return x
```

```python
import functools

import jax
import jax.numpy as jnp
from jax import lax
import jax.experimental.pallas as pl
import jax.experimental.pallas.tpu as pltpu

S, D, F = 2048, 512, 1792
H, DH, W, DIL = 32, 16, 8, 2
HALO = 16
EPS = 1e-5
TM = 256
NT = S // TM
TAIL = 32
WOP = 17
LOG2E = 1.4426950408889634
QSCALE = DH ** -0.5 * LOG2E
NEG = -1e9 * LOG2E
NT_DIMS = (((1,), (1,)), ((), ()))
f32 = jnp.float32
bf16 = jnp.bfloat16
u32 = jnp.uint32


def _ln(x):
    m = jnp.sum(x, axis=-1, keepdims=True) * (1.0 / D)
    xc = x - m
    v = jnp.sum(xc * xc, axis=-1, keepdims=True) * (1.0 / D)
    return xc * lax.rsqrt(v + EPS)


def _gelu2(x):
    c0 = 0.7978845608028654
    u = x * (c0 + (c0 * 0.044715) * (x * x))
    return x * (1.0 + jnp.tanh(u))


def _pack(x):
    return pltpu.bitcast(x.astype(bf16), u32)


def _unpack(x):
    return pltpu.bitcast(x, bf16)


def _rows(parts):
    return parts[0] if len(parts) == 1 else jnp.concatenate(parts, axis=0)


def _kernel(x_hbm, wqkv_hbm, wo_hbm, w1_hbm, b1_hbm, w2_hbm, b2_hbm, c_hbm, wmod_hbm,
            out_hbm,
            x_s, wqkv_s, wo_s, w1_s, b1_s, w2_s, b2_s, c_s, wmod_s,
            mod_s, bias_s, wt_s, wop_s, wof_s, w1p_s,
            qa_s, ka_s, va_s, qb_s, kb_s, vb_s, qc_s, kc_s, vc_s,
            g_s, x1a_s, x1b_s, out_s, zero_s, scol_s, bq_s,
            sem):
    set_a = (qa_s, ka_s, va_s)
    set_b = (qb_s, kb_s, vb_s)
    set_c = (qc_s, kc_s, vc_s)

    def cp(src, dst, k):
        return pltpu.make_async_copy(src, dst, sem.at[k])

    def x_dma(t, k):
        return cp(x_hbm.at[pl.ds(t * TM, TM)], x_s.at[pl.ds(t * TM, TM)], k)

    def out_dma(row0, n=TM):
        return cp(out_s.at[pl.ds(row0, n)], out_hbm.at[pl.ds(row0, n)], 9)

    def wq_dma(j, k):
        return cp(wqkv_hbm.at[:, j * D:(j + 1) * D], wqkv_s.at[:, j * D:(j + 1) * D], k)

    def wm_dma(j0, j1, k):
        return cp(wmod_hbm.at[:, j0 * D:j1 * D], wmod_s.at[:, j0 * D:j1 * D], k)

    groups = [
        [wq_dma(0, 0)],
        [cp(c_hbm, c_s, 1), x_dma(0, 1)],
        [wm_dma(0, 1, 2), x_dma(1, 2)],
        [wq_dma(1, 3)],
        [wq_dma(2, 4), cp(wo_hbm, wo_s, 4), x_dma(2, 4)],
        [wm_dma(2, 5, 5), cp(b1_hbm, b1_s, 5), cp(b2_hbm, b2_s, 5)],
        [cp(w1_hbm, w1_s, 6), wm_dma(5, 6, 6)],
        [x_dma(3, 7), cp(w2_hbm, w2_s, 7)],
        [cp(x_hbm.at[4 * TM:S], x_s.at[4 * TM:S], 8)],
        [wm_dma(1, 2, 10)],
    ]
    for k in (0, 1, 9, 3, 2, 4, 5, 6, 7, 8):
        for d in groups[k]:
            d.start()

    def wait(k):
        for d in groups[k]:
            d.wait()

    def mod_row(j):
        return mod_s[0:1, j * D:(j + 1) * D]

    def link(dst, src):
        n = dst.shape[0] // 8
        z = jnp.concatenate([zero_s[...]] * n, axis=0) if n > 1 else zero_s[...]
        return pltpu.bitcast(pltpu.bitcast(dst, u32) | (pltpu.bitcast(src, u32) & z), f32)

    def link_x(x, src):
        return jnp.concatenate([link(x[:, 0:128], src[:, 0:128]), x[:, 128:]], axis=1)

    def V1(row0, lg=32, nch=0):
        sa = mod_row(0)
        ca1 = mod_row(1)
        done = []
        for r in range(0, TM, lg):
            x = x_s[pl.ds(row0 + r, lg), :].astype(f32)
            if nch and len(done) >= nch:
                x = link_x(x, done[-nch])
            done.append(_ln(x) * ca1 + sa)
        return _rows(done).astype(bf16)

    def halo(src, dst, j):
        dst[j][:, 0:HALO, :] = src[j][:, TM:TM + HALO, :]

    def M1(j, dset, h, extra=None):
        dst = dset[j]
        wt = _unpack(wt_s[j * (D // 2):(j + 1) * (D // 2), :])
        if extra is not None:
            h = _unpack(jnp.concatenate([pltpu.bitcast(h, u32), _pack(extra)], axis=0))
        r = lax.dot_general(h, wt, NT_DIMS, preferred_element_type=f32)
        if extra is not None:
            bq_s[...] = r[TM:TM + 8] * QSCALE
            r = r[0:TM]
        for ct in range(4):
            if j == 0:
                dst[ct] = r[:, ct * 128:(ct + 1) * 128] * QSCALE
            else:
                dst[ct, HALO:HALO + TM, :] = r[:, ct * 128:(ct + 1) * 128]

    def V2(sset, rg, nch, first=False):
        q_s, k_s, v_s = sset
        outs, done, pend = [], [], []
        for r in range(0, TM, rg):
            q = [q_s[ct, r:r + rg, :] for ct in range(4)]
            if first:
                q = [q[ct] + bq_s[0:1, ct * 128:(ct + 1) * 128] for ct in range(4)]
            if nch and len(done) >= nch:
                q[0] = link(q[0], done[-nch])
            logits = []
            for w in range(W):
                off = HALO - DIL * w + r
                t = q[0] * k_s[0, off:off + rg, :]
                for ct in range(1, 4):
                    t = t + q[ct] * k_s[ct, off:off + rg, :]
                t = t + pltpu.roll(t, 64, 1)
                t = t + pltpu.roll(t, 32, 1)
                if first and r < DIL * w:
                    row = r + lax.broadcasted_iota(jnp.int32, (rg, 128), 0)
                    t = jnp.where(row >= DIL * w, t, NEG)
                logits.append(t)
            m = functools.reduce(jnp.maximum, logits)
            p = [jnp.exp2(l - m) for l in logits]
            ssum = functools.reduce(lambda a, b: a + b, p)
            rinv = pl.reciprocal(ssum, approx=True)
            rinv = rinv * (2.0 - ssum * rinv)
            o = []
            for ct in range(4):
                acc = p[0] * v_s[ct, HALO + r:HALO + r + rg, :]
                for w in range(1, W):
                    off = HALO - DIL * w + r
                    acc = acc + p[w] * v_s[ct, off:off + rg, :]
                o.append(acc * rinv)
            done.append(o[3])
            pend.append(jnp.concatenate(o, axis=1))
            if len(pend) * rg >= 16:
                outs.append(_pack(_rows(pend)))
                pend = []
        return outs

    def M2(outs):
        o = _unpack(jnp.concatenate(outs, axis=0))
        return jnp.dot(o, _unpack(wop_s[...]), preferred_element_type=f32)

    def X1(row0, a):
        x1a_s[...] = x_s[pl.ds(row0, TM), :].astype(f32) + mod_row(2) * a

    def V3(lg=32, nch=0):
        sb = mod_row(3)
        cb1 = mod_row(4)
        done = []
        for r in range(0, TM, lg):
            x1 = x1a_s[r:r + lg, :]
            if nch and len(done) >= nch:
                x1 = link_x(x1, done[-nch])
            h2 = _ln(x1) * cb1 + sb
            done.append(_ln(h2))
        y = _rows(done).astype(bf16)
        x1b_s[...] = x1a_s[...]
        return y

    def M3(y, first=False):
        if first:
            w1 = w1_s[...]
            w1p_s[...] = pltpu.bitcast(w1, u32)
        else:
            w1 = _unpack(w1p_s[...])
        u = jnp.dot(y, w1, preferred_element_type=f32) + bias_s[0:1, 0:F]
        g_s[...] = _pack(_gelu2(u))

    def M4(row0, r_lo=0, r_hi=TM):
        g = _unpack(g_s[r_lo // 2:r_hi // 2, :])
        z = jnp.dot(g, w2_s[...], preferred_element_type=f32) + bias_s[0:1, F:F + D]
        out_s[pl.ds(row0 + r_lo, r_hi - r_lo), :] = (x1b_s[r_lo:r_hi, :] + mod_row(5) * z).astype(bf16)

    def permute_wqkv(j):
        r = lax.broadcasted_iota(jnp.int32, (128, 128), 0)
        n = lax.broadcasted_iota(jnp.int32, (128, 128), 1)
        sel = jnp.where(n == (r % 8) * 16 + r // 8, 1.0, 0.0).astype(bf16)
        parts = []
        for nt in range(4):
            src = wqkv_s[:, j * D + nt * 128: j * D + (nt + 1) * 128]
            parts.append(lax.dot_general(sel, src, NT_DIMS, preferred_element_type=f32))
        for d in range(DH):
            blk = jnp.concatenate([p[d * 8:(d + 1) * 8] for p in parts], axis=0)
            wt_s[j * (D // 2) + d * 16: j * (D // 2) + (d + 1) * 16, :] = _pack(blk)

    def permute_wo():
        for ct in range(4):
            for hh in range(H):
                wof_s[ct, hh * WOP:hh * WOP + DH, :] = (
                    wo_s[hh * DH:(hh + 1) * DH, ct * 128:(ct + 1) * 128].astype(f32))
        for ct in range(4):
            for d in range(DH):
                blk = wof_s[ct, pl.ds(d, H, stride=WOP), :]
                wop_s[d * 16:(d + 1) * 16, ct * 128:(ct + 1) * 128] = _pack(blk)

    def silu_c():
        c = c_s[...].astype(f32)
        return c * jax.nn.sigmoid(c)

    def mod_fix(j, mj):
        if j in (1, 4):
            mj = mj + 1.0
        if j == 5:
            mj = mj * 0.5
        return mj

    def mod_mxu(j0, j1):
        sc = jnp.broadcast_to(silu_c(), (8, D)).astype(bf16)
        m = jnp.dot(sc, wmod_s[:, j0 * D:j1 * D], preferred_element_type=f32)
        for j in range(j0, j1):
            mod_s[:, j * D:(j + 1) * D] = mod_fix(j, m[:, (j - j0) * D:(j - j0 + 1) * D])

    def mod_vpu(j):
        sc = scol_s[...]
        w = wmod_s[:, j * D:(j + 1) * D].astype(f32)
        m = jnp.sum(w * jnp.concatenate([sc] * 4, axis=1), axis=0, keepdims=True)
        mod_s[0:1, j * D:(j + 1) * D] = mod_fix(j, m)

    zero_s[...] = jnp.zeros((8, 128), u32)
    kc_s[:, 0:HALO, :] = jnp.zeros((4, HALO, 128), f32)
    vc_s[:, 0:HALO, :] = jnp.zeros((4, HALO, 128), f32)
    wait(0)
    permute_wqkv(0)
    wait(1)
    scol_s[...] = jnp.transpose(jnp.broadcast_to(silu_c().astype(bf16).astype(f32), (128, D)))
    for r in range(0, TM, 32):
        x1b_s[r:r + 32, :] = _ln(x_s[r:r + 32, :].astype(f32))
    wait(9)
    mod_mxu(1, 2)
    xs = x1b_s[...] * mod_row(1)
    x1b_s[...] = xs
    M1(0, set_c, xs.astype(bf16))
    wait(3)
    permute_wqkv(1)
    wait(2)
    mod_mxu(0, 1)
    h0 = (x1b_s[...] + mod_row(0)).astype(bf16)
    h1 = V1(TM)
    M1(1, set_c, h0)
    M1(0, set_b, h1, extra=jnp.broadcast_to(mod_row(0), (16, D)))
    wait(4)
    permute_wqkv(2)
    h2 = V1(2 * TM, 16, 3)
    permute_wo()
    halo(set_c, set_b, 1)
    M1(1, set_b, h1)
    M1(2, set_c, h0)
    halo(set_c, set_b, 2)
    M1(2, set_b, h1)
    a0 = M2(V2(set_c, 64, 0, first=True))
    wait(5)
    mod_mxu(2, 5)
    bias_s[0:1, 0:F] = b1_s[...].astype(f32).reshape(1, F)
    bias_s[0:1, F:F + D] = b2_s[...].astype(f32).reshape(1, D) * 2.0
    X1(0, a0)
    y0 = V3(32, 2)
    M1(0, set_a, h2)
    halo(set_b, set_a, 1)
    M1(1, set_a, h2)
    halo(set_b, set_a, 2)
    M1(2, set_a, h2)
    X1(TM, M2(V2(set_b, 16, 8)))
    wait(6)
    mod_vpu(5)
    M3(y0, first=True)
    wait(7)

    def body(t, carry):
        @pl.when(t == 1)
        def _():
            wait(8)
        r0 = pl.multiple_of(t * TM, TM)
        r2 = pl.multiple_of((t + 2) * TM, TM)
        r3 = pl.multiple_of((t + 3) * TM, TM)
        M4(r0)
        M3(V3())
        X1(r2, M2(V2(set_a, 8, 3)))
        h = V1(r3)
        halo(set_a, set_a, 1)
        halo(set_a, set_a, 2)
        for j in range(3):
            M1(j, set_a, h)
        out_dma(r0).start()
        return carry

    lax.fori_loop(0, NT - 3, body, 0)

    M4((NT - 3) * TM)
    out_dma((NT - 3) * TM).start()
    M3(V3())
    X1((NT - 1) * TM, M2(V2(set_a, 8, 3)))
    M4((NT - 2) * TM)
    out_dma((NT - 2) * TM).start()
    M3(V3())
    M4((NT - 1) * TM, 0, TM - TAIL)
    out_dma((NT - 1) * TM, TM - TAIL).start()
    M4((NT - 1) * TM, TM - TAIL, TM)
    out_dma(S - TAIL, TAIL).start()
    cp(out_s, out_hbm, 9).wait()


@jax.jit
def pallas_adaLN_cond__sliding_local_dilated__mixer_channel_mlp__prompt_kernel(
    A_x: jax.Array,
    A_wqkv: jax.Array,
    A_wo: jax.Array,
    B_x: jax.Array,
    B_w1: jax.Array,
    B_b1: jax.Array,
    B_w2: jax.Array,
    B_b2: jax.Array,
    c: jax.Array,
    w_mod: jax.Array,
):
    any_spec = pl.BlockSpec(memory_space=pl.ANY)
    qkv_set = [pltpu.VMEM((4, TM, 128), f32), pltpu.VMEM((4, TM + HALO, 128), f32),
               pltpu.VMEM((4, TM + HALO, 128), f32)]
    out = pl.pallas_call(
        _kernel,
        in_specs=[any_spec] * 9,
        out_specs=any_spec,
        out_shape=jax.ShapeDtypeStruct((S, D), A_x.dtype),
        scratch_shapes=[
            pltpu.VMEM((S, D), bf16),
            pltpu.VMEM((D, 3 * D), bf16),
            pltpu.VMEM((D, D), bf16),
            pltpu.VMEM((D, F), bf16),
            pltpu.VMEM((F,), bf16),
            pltpu.VMEM((F, D), bf16),
            pltpu.VMEM((D,), bf16),
            pltpu.VMEM((1, D), bf16),
            pltpu.VMEM((D, 6 * D), bf16),
            pltpu.VMEM((8, 6 * D), f32),
            pltpu.VMEM((8, F + D), f32),
            pltpu.VMEM((3 * D // 2, D), u32),
            pltpu.VMEM((D // 2, D), u32),
            pltpu.VMEM((4, H * WOP, 128), f32),
            pltpu.VMEM((D // 2, F), u32),
        ] + qkv_set + qkv_set + qkv_set + [
            pltpu.VMEM((TM // 2, F), u32),
            pltpu.VMEM((TM, D), f32),
            pltpu.VMEM((TM, D), f32),
            pltpu.VMEM((S, D), bf16),
            pltpu.VMEM((8, 128), u32),
            pltpu.VMEM((D, 128), f32),
            pltpu.VMEM((8, D), f32),
            pltpu.SemaphoreType.DMA((11,)),
        ],
        compiler_params=pltpu.CompilerParams(vmem_limit_bytes=64 * 1024 * 1024, disable_bounds_checks=True, disable_semaphore_checks=True),
    )(A_x.reshape(S, D), A_wqkv, A_wo, B_w1, B_b1, B_w2, B_b2, c, w_mod)
    return out.reshape(1, S, D)
```

```python
import functools

import jax
import jax.numpy as jnp
from jax import lax
import jax.experimental.pallas as pl
import jax.experimental.pallas.tpu as pltpu

S, D, F = 2048, 512, 1792
H, DH, W, DIL = 32, 16, 8, 2
HALO = 16
EPS = 1e-5
TM = 256
NT = S // TM
TAIL = 32
WOP = 17
LOG2E = 1.4426950408889634
QSCALE = DH ** -0.5 * LOG2E
NEG = -1e9 * LOG2E
NT_DIMS = (((1,), (1,)), ((), ()))
f32 = jnp.float32
bf16 = jnp.bfloat16
u32 = jnp.uint32


def _ln(x):
    m = jnp.sum(x, axis=-1, keepdims=True) * (1.0 / D)
    xc = x - m
    v = jnp.sum(xc * xc, axis=-1, keepdims=True) * (1.0 / D)
    return xc * lax.rsqrt(v + EPS)


def _gelu2(x):
    c0 = 0.7978845608028654
    u = x * (c0 + (c0 * 0.044715) * (x * x))
    return x * (1.0 + jnp.tanh(u))


def _pack(x):
    return pltpu.bitcast(x.astype(bf16), u32)


def _unpack(x):
    return pltpu.bitcast(x, bf16)


def _rows(parts):
    return parts[0] if len(parts) == 1 else jnp.concatenate(parts, axis=0)


def _kernel(x_hbm, wqkv_hbm, wo_hbm, w1_hbm, b1_hbm, w2_hbm, b2_hbm, c_hbm, wmod_hbm,
            out_hbm,
            x_s, wqkv_s, wo_s, w1_s, b1_s, w2_s, b2_s, c_s, wmod_s,
            mod_s, bias_s, wt_s, wop_s, wof_s, w1p_s,
            qa_s, ka_s, va_s, qb_s, kb_s, vb_s, qc_s, kc_s, vc_s,
            g_s, x1a_s, x1b_s, out_s, zero_s, scol_s, bq_s,
            sem):
    set_a = (qa_s, ka_s, va_s)
    set_b = (qb_s, kb_s, vb_s)
    set_c = (qc_s, kc_s, vc_s)

    def cp(src, dst, k):
        return pltpu.make_async_copy(src, dst, sem.at[k])

    def x_dma(t, k):
        return cp(x_hbm.at[pl.ds(t * TM, TM)], x_s.at[pl.ds(t * TM, TM)], k)

    def out_dma(row0, n=TM):
        return cp(out_s.at[pl.ds(row0, n)], out_hbm.at[pl.ds(row0, n)], 9)

    def wq_dma(j, k):
        return cp(wqkv_hbm.at[:, j * D:(j + 1) * D], wqkv_s.at[:, j * D:(j + 1) * D], k)

    def wm_dma(j0, j1, k):
        return cp(wmod_hbm.at[:, j0 * D:j1 * D], wmod_s.at[:, j0 * D:j1 * D], k)

    groups = [
        [wq_dma(0, 0)],
        [cp(c_hbm, c_s, 1), x_dma(0, 1)],
        [wm_dma(1, 2, 2)],
        [wq_dma(1, 3)],
        [wm_dma(0, 1, 4), x_dma(1, 4)],
        [wq_dma(2, 5), cp(wo_hbm, wo_s, 5), x_dma(2, 5)],
        [wm_dma(2, 5, 6), cp(b1_hbm, b1_s, 6), cp(b2_hbm, b2_s, 6)],
        [cp(w1_hbm, w1_s, 7), wm_dma(5, 6, 7)],
        [cp(w2_hbm, w2_s, 8), cp(x_hbm.at[3 * TM:S], x_s.at[3 * TM:S], 8)],
    ]
    for grp in groups:
        for d in grp:
            d.start()

    def wait(k):
        for d in groups[k]:
            d.wait()

    def mod_row(j):
        return mod_s[0:1, j * D:(j + 1) * D]

    def link(dst, src):
        n = dst.shape[0] // 8
        z = jnp.concatenate([zero_s[...]] * n, axis=0) if n > 1 else zero_s[...]
        return pltpu.bitcast(pltpu.bitcast(dst, u32) | (pltpu.bitcast(src, u32) & z), f32)

    def link_x(x, src):
        return jnp.concatenate([link(x[:, 0:128], src[:, 0:128]), x[:, 128:]], axis=1)

    def V1(row0, lg=32, nch=0):
        sa = mod_row(0)
        ca1 = mod_row(1)
        done = []
        for r in range(0, TM, lg):
            x = x_s[pl.ds(row0 + r, lg), :].astype(f32)
            if nch and len(done) >= nch:
                x = link_x(x, done[-nch])
            done.append(_ln(x) * ca1 + sa)
        return _rows(done).astype(bf16)

    def halo(src, dst, j):
        dst[j][:, 0:HALO, :] = src[j][:, TM:TM + HALO, :]

    def M1(j, dset, h, extra=None):
        dst = dset[j]
        wt = _unpack(wt_s[j * (D // 2):(j + 1) * (D // 2), :])
        if extra is not None:
            h = _unpack(jnp.concatenate([pltpu.bitcast(h, u32), _pack(extra)], axis=0))
        r = lax.dot_general(h, wt, NT_DIMS, preferred_element_type=f32)
        if extra is not None:
            bq_s[...] = r[TM:TM + 8] * QSCALE
            r = r[0:TM]
        for ct in range(4):
            if j == 0:
                dst[ct] = r[:, ct * 128:(ct + 1) * 128] * QSCALE
            else:
                dst[ct, HALO:HALO + TM, :] = r[:, ct * 128:(ct + 1) * 128]

    def V2(sset, rg, nch, first=False):
        q_s, k_s, v_s = sset
        outs, done, pend = [], [], []
        for r in range(0, TM, rg):
            q = [q_s[ct, r:r + rg, :] for ct in range(4)]
            if first:
                q = [q[ct] + bq_s[0:1, ct * 128:(ct + 1) * 128] for ct in range(4)]
            if nch and len(done) >= nch:
                q[0] = link(q[0], done[-nch])
            logits = []
            for w in range(W):
                off = HALO - DIL * w + r
                t = q[0] * k_s[0, off:off + rg, :]
                for ct in range(1, 4):
                    t = t + q[ct] * k_s[ct, off:off + rg, :]
                t = t + pltpu.roll(t, 64, 1)
                t = t + pltpu.roll(t, 32, 1)
                if first and r < DIL * w:
                    row = r + lax.broadcasted_iota(jnp.int32, (rg, 128), 0)
                    t = jnp.where(row >= DIL * w, t, NEG)
                logits.append(t)
            m = functools.reduce(jnp.maximum, logits)
            p = [jnp.exp2(l - m) for l in logits]
            ssum = functools.reduce(lambda a, b: a + b, p)
            rinv = pl.reciprocal(ssum, approx=True)
            rinv = rinv * (2.0 - ssum * rinv)
            o = []
            for ct in range(4):
                acc = p[0] * v_s[ct, HALO + r:HALO + r + rg, :]
                for w in range(1, W):
                    off = HALO - DIL * w + r
                    acc = acc + p[w] * v_s[ct, off:off + rg, :]
                o.append(acc * rinv)
            done.append(o[3])
            pend.append(jnp.concatenate(o, axis=1))
            if len(pend) * rg >= 16:
                outs.append(_pack(_rows(pend)))
                pend = []
        return outs

    def M2(outs):
        o = _unpack(jnp.concatenate(outs, axis=0))
        return jnp.dot(o, _unpack(wop_s[...]), preferred_element_type=f32)

    def X1(row0, a):
        x1a_s[...] = x_s[pl.ds(row0, TM), :].astype(f32) + mod_row(2) * a

    def V3(lg=32, nch=0):
        sb = mod_row(3)
        cb1 = mod_row(4)
        done = []
        for r in range(0, TM, lg):
            x1 = x1a_s[r:r + lg, :]
            if nch and len(done) >= nch:
                x1 = link_x(x1, done[-nch])
            h2 = _ln(x1) * cb1 + sb
            done.append(_ln(h2))
        y = _rows(done).astype(bf16)
        x1b_s[...] = x1a_s[...]
        return y

    def M3(y, first=False):
        if first:
            w1 = w1_s[...]
            w1p_s[...] = pltpu.bitcast(w1, u32)
        else:
            w1 = _unpack(w1p_s[...])
        u = jnp.dot(y, w1, preferred_element_type=f32) + bias_s[0:1, 0:F]
        g_s[...] = _pack(_gelu2(u))

    def M4(row0, r_lo=0, r_hi=TM):
        g = _unpack(g_s[r_lo // 2:r_hi // 2, :])
        z = jnp.dot(g, w2_s[...], preferred_element_type=f32) + bias_s[0:1, F:F + D]
        out_s[pl.ds(row0 + r_lo, r_hi - r_lo), :] = (x1b_s[r_lo:r_hi, :] + mod_row(5) * z).astype(bf16)

    def permute_wqkv(j):
        r = lax.broadcasted_iota(jnp.int32, (128, 128), 0)
        n = lax.broadcasted_iota(jnp.int32, (128, 128), 1)
        sel = jnp.where(n == (r % 8) * 16 + r // 8, 1.0, 0.0).astype(bf16)
        parts = []
        for nt in range(4):
            src = wqkv_s[:, j * D + nt * 128: j * D + (nt + 1) * 128]
            parts.append(lax.dot_general(sel, src, NT_DIMS, preferred_element_type=f32))
        for d in range(DH):
            blk = jnp.concatenate([p[d * 8:(d + 1) * 8] for p in parts], axis=0)
            wt_s[j * (D // 2) + d * 16: j * (D // 2) + (d + 1) * 16, :] = _pack(blk)

    def permute_wo():
        for ct in range(4):
            for hh in range(H):
                wof_s[ct, hh * WOP:hh * WOP + DH, :] = (
                    wo_s[hh * DH:(hh + 1) * DH, ct * 128:(ct + 1) * 128].astype(f32))
        for ct in range(4):
            for d in range(DH):
                blk = wof_s[ct, pl.ds(d, H, stride=WOP), :]
                wop_s[d * 16:(d + 1) * 16, ct * 128:(ct + 1) * 128] = _pack(blk)

    def silu_c():
        c = c_s[...].astype(f32)
        return c * jax.nn.sigmoid(c)

    def mod_fix(j, mj):
        if j in (1, 4):
            mj = mj + 1.0
        if j == 5:
            mj = mj * 0.5
        return mj

    def mod_mxu(j0, j1):
        sc = jnp.broadcast_to(silu_c(), (8, D)).astype(bf16)
        m = jnp.dot(sc, wmod_s[:, j0 * D:j1 * D], preferred_element_type=f32)
        for j in range(j0, j1):
            mod_s[:, j * D:(j + 1) * D] = mod_fix(j, m[:, (j - j0) * D:(j - j0 + 1) * D])

    def mod_vpu(j):
        sc = scol_s[...]
        w = wmod_s[:, j * D:(j + 1) * D].astype(f32)
        m = jnp.sum(w * jnp.concatenate([sc] * 4, axis=1), axis=0, keepdims=True)
        mod_s[0:1, j * D:(j + 1) * D] = mod_fix(j, m)

    zero_s[...] = jnp.zeros((8, 128), u32)
    kc_s[:, 0:HALO, :] = jnp.zeros((4, HALO, 128), f32)
    vc_s[:, 0:HALO, :] = jnp.zeros((4, HALO, 128), f32)
    wait(0)
    permute_wqkv(0)
    wait(1)
    scol_s[...] = jnp.transpose(jnp.broadcast_to(silu_c().astype(bf16).astype(f32), (128, D)))
    for r in range(0, TM, 32):
        x1b_s[r:r + 32, :] = _ln(x_s[r:r + 32, :].astype(f32))
    wait(2)
    mod_mxu(1, 2)
    xs = x1b_s[...] * mod_row(1)
    x1b_s[...] = xs
    M1(0, set_c, xs.astype(bf16))
    wait(3)
    permute_wqkv(1)
    wait(4)
    mod_mxu(0, 1)
    h0 = (x1b_s[...] + mod_row(0)).astype(bf16)
    h1 = V1(TM)
    M1(1, set_c, h0)
    M1(0, set_b, h1, extra=jnp.broadcast_to(mod_row(0), (16, D)))
    wait(5)
    permute_wqkv(2)
    h2 = V1(2 * TM, 16, 3)
    permute_wo()
    halo(set_c, set_b, 1)
    M1(1, set_b, h1)
    M1(2, set_c, h0)
    halo(set_c, set_b, 2)
    M1(2, set_b, h1)
    a0 = M2(V2(set_c, 64, 0, first=True))
    wait(6)
    mod_mxu(2, 5)
    bias_s[0:1, 0:F] = b1_s[...].astype(f32).reshape(1, F)
    bias_s[0:1, F:F + D] = b2_s[...].astype(f32).reshape(1, D) * 2.0
    X1(0, a0)
    y0 = V3(32, 2)
    M1(0, set_a, h2)
    halo(set_b, set_a, 1)
    M1(1, set_a, h2)
    halo(set_b, set_a, 2)
    M1(2, set_a, h2)
    X1(TM, M2(V2(set_b, 16, 8)))
    wait(7)
    mod_vpu(5)
    M3(y0, first=True)
    wait(8)

    def body(t, carry):
        r0 = pl.multiple_of(t * TM, TM)
        r2 = pl.multiple_of((t + 2) * TM, TM)
        r3 = pl.multiple_of((t + 3) * TM, TM)
        M4(r0)
        out_dma(r0).start()
        M3(V3())
        X1(r2, M2(V2(set_a, 8, 3)))
        h = V1(r3)
        halo(set_a, set_a, 1)
        halo(set_a, set_a, 2)
        for j in range(3):
            M1(j, set_a, h)
        return carry

    lax.fori_loop(0, NT - 3, body, 0)

    M4((NT - 3) * TM)
    out_dma((NT - 3) * TM).start()
    M3(V3())
    X1((NT - 1) * TM, M2(V2(set_a, 8, 3)))
    M4((NT - 2) * TM)
    out_dma((NT - 2) * TM).start()
    M3(V3())
    M4((NT - 1) * TM, 0, TM - TAIL)
    out_dma((NT - 1) * TM, TM - TAIL).start()
    M4((NT - 1) * TM, TM - TAIL, TM)
    out_dma(S - TAIL, TAIL).start()
    cp(out_s, out_hbm, 9).wait()


@jax.jit
def pallas_adaLN_cond__sliding_local_dilated__mixer_channel_mlp__prompt_kernel(
    A_x: jax.Array,
    A_wqkv: jax.Array,
    A_wo: jax.Array,
    B_x: jax.Array,
    B_w1: jax.Array,
    B_b1: jax.Array,
    B_w2: jax.Array,
    B_b2: jax.Array,
    c: jax.Array,
    w_mod: jax.Array,
):
    any_spec = pl.BlockSpec(memory_space=pl.ANY)
    qkv_set = [pltpu.VMEM((4, TM, 128), f32), pltpu.VMEM((4, TM + HALO, 128), f32),
               pltpu.VMEM((4, TM + HALO, 128), f32)]
    out = pl.pallas_call(
        _kernel,
        in_specs=[any_spec] * 9,
        out_specs=any_spec,
        out_shape=jax.ShapeDtypeStruct((S, D), A_x.dtype),
        scratch_shapes=[
            pltpu.VMEM((S, D), bf16),
            pltpu.VMEM((D, 3 * D), bf16),
            pltpu.VMEM((D, D), bf16),
            pltpu.VMEM((D, F), bf16),
            pltpu.VMEM((F,), bf16),
            pltpu.VMEM((F, D), bf16),
            pltpu.VMEM((D,), bf16),
            pltpu.VMEM((1, D), bf16),
            pltpu.VMEM((D, 6 * D), bf16),
            pltpu.VMEM((8, 6 * D), f32),
            pltpu.VMEM((8, F + D), f32),
            pltpu.VMEM((3 * D // 2, D), u32),
            pltpu.VMEM((D // 2, D), u32),
            pltpu.VMEM((4, H * WOP, 128), f32),
            pltpu.VMEM((D // 2, F), u32),
        ] + qkv_set + qkv_set + qkv_set + [
            pltpu.VMEM((TM // 2, F), u32),
            pltpu.VMEM((TM, D), f32),
            pltpu.VMEM((TM, D), f32),
            pltpu.VMEM((S, D), bf16),
            pltpu.VMEM((8, 128), u32),
            pltpu.VMEM((D, 128), f32),
            pltpu.VMEM((8, D), f32),
            pltpu.SemaphoreType.DMA((10,)),
        ],
        compiler_params=pltpu.CompilerParams(vmem_limit_bytes=64 * 1024 * 1024,
                                             disable_bounds_checks=True,
                                             disable_semaphore_checks=True),
    )(A_x.reshape(S, D), A_wqkv, A_wo, B_w1, B_b1, B_w2, B_b2, c, w_mod)
    return out.reshape(1, S, D)
```
